```python
import os as _os
_os.environ.setdefault("JAX_PLATFORMS", "cpu")
import jax
import jax.numpy as jnp

def _softmax(x, axis=-1):
    return jax.nn.softmax(x, axis=axis)
def _gelu(x):
    return jax.nn.gelu(x, approximate=True)
def _silu(x):
    return jax.nn.silu(x)
def _sigmoid(x):
    return jax.nn.sigmoid(x)
def _layernorm(x, axis=-1, eps=1e-5):
    m = jnp.mean(x, axis=axis, keepdims=True)
    v = jnp.var(x, axis=axis, keepdims=True)
    return (x - m) / jnp.sqrt(v + eps)
def _scatter_add(tgt, idx, src, axis=0):
    return tgt.at[idx].add(src)
def _segment_sum(src, seg, n):
    return jax.ops.segment_sum(src, seg, n)
class _Rng:
    def __init__(self, key):
        self._k = key
    def _next(self):
        self._k, sub = jax.random.split(self._k)
        return sub
    def normal(self, shape):
        return jax.random.normal(self._next(), shape, dtype=jnp.bfloat16)
    def randint(self, lo, hi, shape):
        return jax.random.randint(self._next(), shape, lo, hi, dtype=jnp.int32)
    def uniform(self, shape, lo=0.0, hi=1.0):
        return jax.random.uniform(self._next(), shape, jnp.bfloat16, lo, hi)
    def permutation(self, n):
        return jax.random.permutation(self._next(), n)


kernel_name = 'interleave_layers__sliding_local_dilated__linear_kernel_hedgehog__prompt'

def setup_inputs():
    _rng = _Rng(jax.random.key(int.from_bytes(__import__("os").urandom(4), "little")))
    _w = (lambda a: (lambda t: t.astype(jnp.bfloat16) if jnp.issubdtype(t.dtype, jnp.floating) else t)(jnp.asarray(a)))
    def _A_setup():
        B, S, D = 1, 2048, 640
        return {
            "x": _w((lambda *s: _rng.normal(s) * 0.05)(B, S, D)),
            "wqkv": _w((lambda *s: _rng.normal(s) * 0.05)(D, 3 * D)),
            "wo": _w((lambda *s: _rng.normal(s) * 0.05)(D, D)),
        }
    _A_in = _A_setup()

    def _B_setup():
        B, S, D, H = 1, 2048, 640, 32
        Dh = D // H
        return {
            "x": _w((lambda *s: _rng.normal(s) * 0.05)(B, S, D)),
            "wqkv": _w((lambda *s: _rng.normal(s) * 0.4)(D, 3 * D)),
            "w_phi": _w((lambda *s: _rng.normal(s) * 0.4)(H, Dh, Dh) * (Dh ** -0.5)),
            "wo": _w((lambda *s: _rng.normal(s) * 0.1)(D, D)),
        }
    _B_in = _B_setup()

    return {
        "A_x": _A_in["x"],
        "A_wqkv": _A_in["wqkv"],
        "A_wo": _A_in["wo"],
        "B_x": _B_in["x"],
        "B_wqkv": _B_in["wqkv"],
        "B_w_phi": _B_in["w_phi"],
        "B_wo": _B_in["wo"],
    }

def reference(A_x, A_wqkv, A_wo, B_x, B_wqkv, B_w_phi, B_wo):
    def _A_ref(x, wqkv, wo):
        B, S, D = x.shape
        H = 32; Dh = D // H
        W, dil = 8, 2
        qkv = (lambda x, *d: x.transpose(*d))((x @ wqkv).reshape(B, S, 3, H, Dh), 2, 0, 3, 1, 4)
        q, k, v = qkv[0], qkv[1], qkv[2]
        scale = Dh ** -0.5
        pos = jnp.arange(S)
        off = jnp.arange(W) * dil
        idx = pos[:, None] - off[None, :]
        mask = idx >= 0
        idx_c = jnp.where(mask, idx, 0).reshape(-1)
        kg = k[:, :, idx_c, :].reshape(B, H, S, W, Dh)
        vg = v[:, :, idx_c, :].reshape(B, H, S, W, Dh)
        logits = jnp.einsum("bhsd,bhswd->bhsw", q, kg) * scale
        logits = jnp.where(mask[None, None, :, :], logits, -1e9)
        attn = _softmax(logits, axis=-1)
        o = jnp.einsum("bhsw,bhswd->bhsd", attn, vg)
        return (lambda x, *d: x.transpose(*d))(o, 0, 2, 1, 3).reshape(B, S, D) @ wo

    def _B_ref(x, wqkv, w_phi, wo):
        B, S, D = x.shape
        H = 32; Dh = D // H
        qkv = (lambda x, *d: x.transpose(*d))((x @ wqkv).reshape(B, S, 3, H, Dh), 2, 0, 3, 1, 4)
        q, k, v = qkv[0], qkv[1], qkv[2]
        pq = jnp.einsum("bhsd,hdf->bhsf", q, w_phi)
        pk = jnp.einsum("bhsd,hdf->bhsf", k, w_phi)
        phi_q = jnp.concatenate([_softmax(pq, axis=-1), _softmax(-pq, axis=-1)], axis=-1)
        phi_k = jnp.concatenate([_softmax(pk, axis=-1), _softmax(-pk, axis=-1)], axis=-1)
        kv = jnp.einsum("bhsf,bhsd->bhfd", phi_k, v)
        z  = jnp.einsum("bhsf->bhf", phi_k)
        num = jnp.einsum("bhqf,bhfd->bhqd", phi_q, kv)
        den = jnp.einsum("bhqf,bhf->bhq", phi_q, z)[..., None] + 1e-6
        o = num / den
        return (lambda x, *d: x.transpose(*d))(o, 0, 2, 1, 3).reshape(B, S, D) @ wo

    x = A_x
    x = x + _A_ref(_layernorm(x, axis=-1), A_wqkv, A_wo)
    x = x + _B_ref(_layernorm(x, axis=-1), B_wqkv, B_w_phi, B_wo)
    x = x + _A_ref(_layernorm(x, axis=-1), A_wqkv, A_wo)
    x = x + _B_ref(_layernorm(x, axis=-1), B_wqkv, B_w_phi, B_wo)
    return x
```

```python
import jax
import jax.numpy as jnp
from jax import lax
import jax.experimental.pallas as pl
import jax.experimental.pallas.tpu as pltpu

S, D, H, DH = 2048, 640, 32, 20
NW = 8
G = 4
GR = 160
CH = 512
NC = S // CH
LOG2E = 1.4426950408889634
F32, BF16 = jnp.float32, jnp.bfloat16


def _nt(a, b):
    return lax.dot_general(a, b, (((1,), (1,)), ((), ())), preferred_element_type=F32)


def _mm(a, b):
    return jnp.dot(a, b, preferred_element_type=F32)


def _tree(fn, xs):
    xs = list(xs)
    while len(xs) > 1:
        xs = [fn(xs[i], xs[i + 1]) if i + 1 < len(xs) else xs[i] for i in range(0, len(xs), 2)]
    return xs[0]


def _layernorm_t(x):
    n = x.shape[1]
    m = jnp.sum(jnp.sum(x.reshape(D // 8, 8, n), axis=0), axis=0, keepdims=True) * (1.0 / D)
    xc = x - m
    v = jnp.sum(jnp.sum((xc * xc).reshape(D // 8, 8, n), axis=0), axis=0, keepdims=True) * (1.0 / D)
    return (xc * lax.rsqrt(v + 1e-5)).astype(BF16)


def kernel(x_hbm, awqkv_hbm, awo_hbm, bwqkv_hbm, wphi_ref, bwo_hbm, out_hbm,
           xin, xin32, wraw, wraw2, woraw, woraw2, tmp, wpf, wa, wb, woa, wob, xt, qs, ks, vs, os_, pq, kv, sems):
    cx = [pltpu.make_async_copy(x_hbm.at[:, pl.ds(i * 128, 128)], xin.at[:, pl.ds(i * 128, 128)], sems.at[5 + i])
          for i in range(5)]
    cwa = pltpu.make_async_copy(awqkv_hbm, wraw, sems.at[1])
    cwoa = pltpu.make_async_copy(awo_hbm, woraw, sems.at[2])
    cwb = pltpu.make_async_copy(bwqkv_hbm, wraw2, sems.at[3])
    cwob = pltpu.make_async_copy(bwo_hbm, woraw2, sems.at[4])
    for c in cx:
        c.start()
    cwa.start()

    for i in range(5):
        cx[i].wait()
        xin32[i] = pltpu.bitcast(xin[:, pl.ds(i * 128, 128)], jnp.uint32)
        for jj in range(8):
            u = xin32[i, pl.ds(jj, 128, stride=8), :].T
            xt[jj, pl.ds(i * 128, 128), :] = pltpu.bitcast(u << 16, F32)
            xt[8 + jj, pl.ds(i * 128, 128), :] = pltpu.bitcast(u & jnp.uint32(0xFFFF0000), F32)

    base = (0, 128, 256, 384)
    row = lax.broadcasted_iota(jnp.int32, (GR, 256), 0)
    col = lax.broadcasted_iota(jnp.int32, (GR, 256), 1)

    def proj_w(src, dst, t, g, p, scale=None):
        w = _nt(p, src[:, pl.ds(t * D + base[g], 256)])
        if scale is not None:
            w = w * scale
        dst[pl.ds(t * D + g * GR, GR), :] = w.astype(BF16)

    def perm(g):
        tgt = (row & 7) * DH + (row >> 3) + (g * GR - base[g])
        return jnp.where(col == tgt, 1.0, 0.0).astype(BF16)

    def xlu_w(src, dst, t):
        for i in range(5):
            u = src[:, pl.ds(t * D + i * 128, 128)].astype(F32).T
            for j in range(5):
                tmp[j, pl.ds(i * 128, 128), :] = u[:, j * 128:(j + 1) * 128]
        for g in range(G):
            for d in range(0, DH, 2):
                r = [jnp.concatenate([tmp[i, pl.ds(g * GR + d + k, 8, stride=DH), :] for i in range(5)], axis=1)
                     for k in range(2)]
                dst[pl.ds(t * D + g * GR + d * 8, 16), :] = jnp.concatenate(r, axis=0).astype(BF16)

    cwa.wait()
    cwoa.start()
    cwb.start()
    cwob.start()
    for g in range(G):
        p = perm(g)
        for t in range(2):
            proj_w(wraw, wa, t, g, p)
    xlu_w(wraw, wa, 2)

    def prep_wo(src, dst):
        for i in range(5):
            tmp[i] = src[:, pl.ds(i * 128, 128)].astype(F32)
        for g in range(G):
            for d in range(DH):
                for i in range(5):
                    vs[i, pl.ds(g * GR + d * 8, 8), :] = tmp[i, pl.ds(g * GR + d, 8, stride=DH), :]
        for i in range(5):
            dst[pl.ds(i * 128, 128), :] = vs[i].T.astype(BF16)

    cwoa.wait()
    prep_wo(woraw, woa)

    cwb.wait()
    wpf[...] = jnp.zeros(wpf.shape, F32)
    for h in range(H):
        wpf[pl.ds(h * DH, DH), pl.ds(0, DH)] = wphi_ref[h].astype(F32)
    srow = lax.broadcasted_iota(jnp.int32, (GR, 128), 0)
    scol = lax.broadcasted_iota(jnp.int32, (GR, 128), 1)
    sel = jnp.where((srow >> 3) == scol, 1.0, 0.0).astype(BF16)
    for g in range(G):
        cc = col - (g * GR - base[g])
        ok = (cc >= 0) & (cc < GR) & ((row & 7) == ((cc * 3277) >> 16))
        p = jnp.where(ok, _nt(sel, wpf[pl.ds(base[g], 256), :].astype(BF16)), 0.0).astype(BF16)
        proj_w(wraw2, wb, 0, g, p, LOG2E)
        proj_w(wraw2, wb, 1, g, p, LOG2E)
    xlu_w(wraw2, wb, 2)
    cwob.wait()
    prep_wo(woraw2, wob)

    lane = lax.broadcasted_iota(jnp.int32, (8, 128), 1)

    def load_x(c):
        return jnp.concatenate([xt[4 * c + i] for i in range(4)], axis=1)

    def add_x(c, y):
        for i in range(4):
            xt[4 * c + i] += y[:, i * 128:(i + 1) * 128]

    def layer_a():
        def proj(c, _):
            y = _mm(wa[...], os_[...])
            os_[...] = _layernorm_t(load_x(jnp.minimum(c + 1, NC - 1)))
            q, k, v = y[:D], y[D:2 * D], y[2 * D:]
            c2 = c // 2
            e0 = c2 * 15 + 7 + (c % 2) * 4
            for i in range(4):
                sl = slice(i * 128, (i + 1) * 128)
                qs[4 * c + i] = q[:, sl]
                ks[e0 + i] = k[:, sl]
                vs[e0 + i] = v[:, sl]
                jj = (c % 2) * 4 + i
                eh = jnp.where(jj == 0, 30, c2 * 15 + jj - 1)
                ks[eh] = pltpu.roll(k[:, sl], 1, 1)
                vs[eh] = pltpu.roll(v[:, sl], 1, 1)
            return _
        os_[...] = _layernorm_t(load_x(0))
        lax.fori_loop(0, NC, proj, 0)

        def attn(c):
            for i in range(4):
                b = 4 * c + i
                jj = (c % 2) * 4 + i
                e0 = (c // 2) * 15 + jj + 7
                for g in range(G):
                    rs = pl.ds(g * GR, GR)
                    q = qs[b, rs, :].reshape(DH, 8, 128)
                    lg = []
                    for w in range(NW):
                        k = ks[e0 - w, rs, :].reshape(DH, 8, 128)
                        l = jnp.sum(q * k, axis=0) * (DH ** -0.5)
                        if w > i:
                            l = jnp.where(jnp.logical_and(lane == 0, jj < w), -1e9, l)
                        lg.append(l)
                    m = _tree(jnp.maximum, lg)
                    ex = [jnp.exp(l - m) for l in lg]
                    r = 1.0 / _tree(jnp.add, ex)
                    o = None
                    for w in range(NW):
                        v = vs[e0 - w, rs, :].reshape(DH, 8, 128)
                        t = v * (ex[w] * r)[None]
                        o = t if o is None else o + t
                    os_[rs, pl.ds(i * 128, 128)] = o.reshape(GR, 128).astype(BF16)
            add_x(c, _mm(woa[...], os_[...]))
        return attn

    def softmax2(p):
        mx = jnp.max(p, axis=0)
        mn = jnp.min(p, axis=0)
        e1 = jnp.exp2(p - mx[None])
        e2 = jnp.exp2(mn[None] - p)
        r1 = 1.0 / jnp.sum(e1, axis=0)
        r2 = 1.0 / jnp.sum(e2, axis=0)
        n = p.shape[-1]
        return ((e1 * r1[None]).reshape(GR, n).astype(BF16), (e2 * r2[None]).reshape(GR, n).astype(BF16))

    def layer_b(attn):
        kv[...] = jnp.zeros(kv.shape, F32)

        def projb(c):
            xn = _layernorm_t(load_x(c))
            ones = jnp.ones((16, CH), BF16)
            for g in range(G):
                q = _mm(wb[pl.ds(g * GR, GR), :], xn)
                k = _mm(wb[pl.ds(D + g * GR, GR), :], xn)
                v = _mm(wb[pl.ds(2 * D + g * GR, GR), :], xn).astype(BF16)
                pk = []
                for i in range(4):
                    sl = slice(i * 128, (i + 1) * 128)
                    a, b = softmax2(q[:, sl].reshape(DH, 8, 128))
                    pq[c, pl.ds(g * 2 * GR, GR), sl] = a
                    pq[c, pl.ds(g * 2 * GR + GR, GR), sl] = b
                    pk.append(softmax2(k[:, sl].reshape(DH, 8, 128)))
                pkc = jnp.concatenate([jnp.concatenate([a for a, _ in pk], axis=1),
                                       jnp.concatenate([b for _, b in pk], axis=1)], axis=0)
                kv[g] += _nt(jnp.concatenate([v, ones], axis=0), pkc)
        attn(0)

        def body(c, _):
            projb(c)
            attn(c + 1)
            return _
        lax.fori_loop(0, NC - 1, body, 0)
        projb(NC - 1)

        r = lax.broadcasted_iota(jnp.int32, (GR + 16, 2 * GR), 0)
        cc = lax.broadcasted_iota(jnp.int32, (GR + 16, 2 * GR), 1)
        msk = (r & 7) == (cc & 7)
        kvb = [jnp.where(msk, kv[g], 0.0).astype(BF16) for g in range(G)]

        def outp(c, _):
            for g in range(G):
                nd = _mm(kvb[g], pq[c, pl.ds(g * 2 * GR, 2 * GR), :])
                rd = 1.0 / (nd[GR:GR + 8] + 1e-6)
                o = nd[:GR].reshape(DH, 8, CH) * rd[None]
                os_[pl.ds(g * GR, GR), :] = o.reshape(GR, CH).astype(BF16)
            add_x(c, _mm(wob[...], os_[...]))
            return _
        lax.fori_loop(0, NC, outp, 0)

    def two(_, carry):
        layer_b(layer_a())
        return carry
    lax.fori_loop(0, 2, two, 0)

    co = [pltpu.make_async_copy(xin.at[:, pl.ds(i * 128, 128)], out_hbm.at[:, pl.ds(i * 128, 128)], sems.at[5 + i])
          for i in range(5)]
    for i in range(5):
        rs = pl.ds(i * 128, 128)
        for jj in range(8):
            ev = pltpu.bitcast(xt[jj, rs, :].astype(BF16).astype(F32), jnp.uint32)
            od = pltpu.bitcast(xt[8 + jj, rs, :].astype(BF16).astype(F32), jnp.uint32)
            xin32[i, pl.ds(jj, 128, stride=8), :] = (od | (ev >> 16)).T
        xin[:, rs] = pltpu.bitcast(xin32[i], BF16)
        co[i].start()
    for c in co:
        c.wait()


@jax.jit
def pallas_interleave_layers__sliding_local_dilated__linear_kernel_hedgehog__prompt_kernel(
    A_x, A_wqkv, A_wo, B_x, B_wqkv, B_w_phi, B_wo,
):
    del B_x
    hbm = pl.BlockSpec(memory_space=pl.ANY)
    out = pl.pallas_call(
        kernel,
        out_shape=jax.ShapeDtypeStruct((S, D), BF16),
        in_specs=[hbm, hbm, hbm, hbm, pl.BlockSpec(memory_space=pltpu.VMEM), hbm],
        out_specs=hbm,
        scratch_shapes=[
            pltpu.VMEM((S, D), BF16),
            pltpu.VMEM((5, S // 2, 128), jnp.uint32),
            pltpu.VMEM((D, 3 * D), BF16),
            pltpu.VMEM((D, 3 * D), BF16),
            pltpu.VMEM((D, D), BF16),
            pltpu.VMEM((D, D), BF16),
            pltpu.VMEM((5, D, 128), F32),
            pltpu.VMEM((D, 128), F32),
            pltpu.VMEM((3 * D, D), BF16),
            pltpu.VMEM((3 * D, D), BF16),
            pltpu.VMEM((D, D), BF16),
            pltpu.VMEM((D, D), BF16),
            pltpu.VMEM((16, D, 128), F32),
            pltpu.VMEM((16, D, 128), F32),
            pltpu.VMEM((31, D, 128), F32),
            pltpu.VMEM((31, D, 128), F32),
            pltpu.VMEM((D, CH), BF16),
            pltpu.VMEM((NC, 2 * D, CH), BF16),
            pltpu.VMEM((G, GR + 16, 2 * GR), F32),
            pltpu.SemaphoreType.DMA((10,)),
        ],
        compiler_params=pltpu.CompilerParams(vmem_limit_bytes=110 * 1024 * 1024),
    )(A_x.reshape(S, D), A_wqkv, A_wo, B_wqkv, B_w_phi, B_wo)
    return out.reshape(1, S, D)
```
